```python
import os as _os
_os.environ.setdefault("JAX_PLATFORMS", "cpu")
import jax
import jax.numpy as jnp

def _softmax(x, axis=-1):
    return jax.nn.softmax(x, axis=axis)
def _gelu(x):
    return jax.nn.gelu(x, approximate=True)
def _silu(x):
    return jax.nn.silu(x)
def _sigmoid(x):
    return jax.nn.sigmoid(x)
def _layernorm(x, axis=-1, eps=1e-5):
    m = jnp.mean(x, axis=axis, keepdims=True)
    v = jnp.var(x, axis=axis, keepdims=True)
    return (x - m) / jnp.sqrt(v + eps)
def _scatter_add(tgt, idx, src, axis=0):
    return tgt.at[idx].add(src)
def _segment_sum(src, seg, n):
    return jax.ops.segment_sum(src, seg, n)
class _Rng:
    def __init__(self, key):
        self._k = key
    def _next(self):
        self._k, sub = jax.random.split(self._k)
        return sub
    def normal(self, shape):
        return jax.random.normal(self._next(), shape, dtype=jnp.bfloat16)
    def randint(self, lo, hi, shape):
        return jax.random.randint(self._next(), shape, lo, hi, dtype=jnp.int32)
    def uniform(self, shape, lo=0.0, hi=1.0):
        return jax.random.uniform(self._next(), shape, jnp.bfloat16, lo, hi)
    def permutation(self, n):
        return jax.random.permutation(self._next(), n)


kernel_name = 'standalone__mha_softmax__near_ridge'

def setup_inputs():
    _rng = _Rng(jax.random.key(int.from_bytes(__import__("os").urandom(4), "little")))
    _w = (lambda a: (lambda t: t.astype(jnp.bfloat16) if jnp.issubdtype(t.dtype, jnp.floating) else t)(jnp.asarray(a)))
    B, H, Sq, Sk, D = 16, 16, 256, 256, 256
    return {
        "q": _w((lambda *s: _rng.normal(s) * 0.4)(B, H, Sq, D)),
        "k": _w((lambda *s: _rng.normal(s) * 0.4)(B, H, Sk, D)),
        "v": _w((lambda *s: _rng.normal(s) * 0.05)(B, H, Sk, D)),
    }

def reference(q, k, v):
    scale = q.shape[-1] ** -0.5
    scores = jnp.einsum("bhqd,bhkd->bhqk", q, k) * scale
    p = _softmax(scores, axis=-1)
    return jnp.einsum("bhqk,bhkd->bhqd", p, v)
```

```python
import jax
import jax.numpy as jnp
import jax.experimental.pallas as pl
import jax.experimental.pallas.tpu as pltpu

_LOG2E = 1.4426950408889634

_HEADS_PER_CHUNK = 2
_NUM_SLOTS = 4
_LAG = 1


def _attention_head(q, k, v, scale):
    s = jax.lax.dot_general(
        q, k, (((1,), (1,)), ((), ())), preferred_element_type=jnp.float32)
    m = jnp.max(s, axis=-1, keepdims=True)
    p = jnp.exp2((s - m) * (scale * _LOG2E))
    l = jnp.sum(p, axis=-1, keepdims=True)
    o = jnp.dot(p.astype(v.dtype), v, preferred_element_type=jnp.float32)
    return (o * pl.reciprocal(l, approx=False)).astype(q.dtype)


@jax.jit
def pallas_standalone__mha_softmax__near_ridge_kernel(
    q: jax.Array,
    k: jax.Array,
    v: jax.Array,
):
    B, H, Sq, D = q.shape
    Sk = k.shape[2]
    n, nb, lag = _HEADS_PER_CHUNK, _NUM_SLOTS, _LAG
    num_heads = B * H
    assert num_heads % n == 0
    G = num_heads // n
    scale = D ** -0.5
    i0 = G - 1 - lag
    assert i0 > 0 and G >= nb

    q3 = q.reshape(num_heads, Sq, D)
    k3 = k.reshape(num_heads, Sk, D)
    v3 = v.reshape(num_heads, Sk, D)

    def kernel(q_hbm, k_hbm, v_hbm, o_hbm, qb, kb, vb, ob, isem, osem, tsem):
        def reads(step, slot):
            return [
                pltpu.make_async_copy(
                    src.at[pl.ds(step * n, n)], dst.at[slot], isem.at[slot, j])
                for j, (src, dst) in enumerate(
                    ((q_hbm, qb), (k_hbm, kb), (v_hbm, vb)))
            ]

        def bulk_write():
            return pltpu.make_async_copy(
                ob.at[pl.ds(0, i0 * n)], o_hbm.at[pl.ds(0, i0 * n)], osem.at[0])

        def tail_write(step):
            return pltpu.make_async_copy(
                ob.at[pl.ds(step * n, n)], o_hbm.at[pl.ds(step * n, n)],
                tsem.at[step - i0])

        def fetch(i):
            @pl.when(i + nb - 1 < G)
            def _():
                for c in reads(i + nb - 1, (i + nb - 1) % nb):
                    c.start()
            for c in reads(i, i % nb):
                c.wait()

        def compute(i):
            slot = i % nb
            for h in range(n):
                ob[i * n + h] = _attention_head(
                    qb[slot, h], kb[slot, h], vb[slot, h], scale)

        for i in range(nb - 1):
            for c in reads(i, i):
                c.start()

        @pl.loop(0, i0)
        def _(i):
            fetch(i)
            compute(i)

        @pl.loop(i0, G)
        def _(i):
            fetch(i)

            @pl.when(i == i0)
            def _():
                bulk_write().start()

            compute(i)
            tail_write(i).start()

        bulk_write().wait()

        @pl.loop(i0, G)
        def _(i):
            tail_write(i).wait()

    hbm = pl.BlockSpec(memory_space=pl.ANY)
    o = pl.pallas_call(
        kernel,
        in_specs=[hbm, hbm, hbm],
        out_specs=hbm,
        out_shape=jax.ShapeDtypeStruct((num_heads, Sq, D), q.dtype),
        scratch_shapes=[
            pltpu.VMEM((nb, n, Sq, D), q.dtype),
            pltpu.VMEM((nb, n, Sk, D), k.dtype),
            pltpu.VMEM((nb, n, Sk, D), v.dtype),
            pltpu.VMEM((num_heads, Sq, D), q.dtype),
            pltpu.SemaphoreType.DMA((nb, 3)),
            pltpu.SemaphoreType.DMA((1,)),
            pltpu.SemaphoreType.DMA((G - i0,)),
        ],
        compiler_params=pltpu.CompilerParams(vmem_limit_bytes=64 * 1024 * 1024),
    )(q3, k3, v3)
    return o.reshape(B, H, Sq, D)
```

```python
import jax
import jax.numpy as jnp
import jax.experimental.pallas as pl
import jax.experimental.pallas.tpu as pltpu

_LOG2E = 1.4426950408889634

_HEADS_PER_CHUNK = 2
_NUM_SLOTS = 4
_PIECE_ROWS = 128
_NUM_PASSES = 32


def _attention_head(q, k, v, scale):
    s = jax.lax.dot_general(
        q, k, (((1,), (1,)), ((), ())), preferred_element_type=jnp.float32)
    m = jnp.max(s, axis=-1, keepdims=True)
    p = jnp.exp2((s - m) * (scale * _LOG2E))
    l = jnp.sum(p, axis=-1, keepdims=True)
    o = jnp.dot(p.astype(v.dtype), v, preferred_element_type=jnp.float32)
    return (o * pl.reciprocal(l, approx=False)).astype(q.dtype)


@jax.jit
def pallas_standalone__mha_softmax__near_ridge_kernel(
    q: jax.Array,
    k: jax.Array,
    v: jax.Array,
):
    B, H, Sq, D = q.shape
    Sk = k.shape[2]
    scale = D ** -0.5
    num_heads = B * H
    n, nb = _HEADS_PER_CHUNK, _NUM_SLOTS
    R, M = _PIECE_ROWS, _NUM_PASSES

    num_chunks = num_heads // n
    pieces_per_head = Sq // R
    heads_per_group = M // pieces_per_head
    num_groups = num_heads // heads_per_group
    assert num_heads % n == 0 and Sq % R == 0 and M % pieces_per_head == 0
    assert num_heads % heads_per_group == 0 and num_chunks >= nb

    start_step = num_chunks - 2
    heads_done = start_step * n
    early_passes = min(
        M, (heads_done - (num_heads - heads_per_group)) * pieces_per_head)
    assert early_passes >= 1

    q3 = q.reshape(num_heads, Sq, D)
    k3 = k.reshape(num_heads, Sk, D)
    v3 = v.reshape(num_heads, Sk, D)

    def kernel(q_hbm, k_hbm, v_hbm, o_hbm, qb, kb, vb, ob, in_sems, out_sem):
        def reads(step, slot):
            return [
                pltpu.make_async_copy(
                    src.at[pl.ds(step * n, n)], dst.at[slot], in_sems.at[slot])
                for src, dst in ((q_hbm, qb), (k_hbm, kb), (v_hbm, vb))
            ]

        def write_pass(j):
            return pltpu.make_async_copy(
                ob.at[:, j], o_hbm.at[:, j], out_sem.at[0])

        for i in range(nb - 1):
            for c in reads(i, i):
                c.start()

        @pl.loop(0, num_chunks)
        def _(i):
            @pl.when(i + nb - 1 < num_chunks)
            def _():
                for c in reads(i + nb - 1, (i + nb - 1) % nb):
                    c.start()

            slot = i % nb
            for c in reads(i, slot):
                c.wait()

            @pl.when(i == start_step)
            def _():
                for j in range(early_passes):
                    write_pass(j).start()

            for h in range(n):
                head = i * n + h
                o = _attention_head(
                    qb[slot, h], kb[slot, h], vb[slot, h], scale)
                ob[head // heads_per_group,
                   pl.ds((head % heads_per_group) * pieces_per_head,
                         pieces_per_head)] = o.reshape(pieces_per_head, R, D)

        for j in range(early_passes, M):
            write_pass(j).start()
        for j in range(M):
            write_pass(j).wait()

    hbm = pl.BlockSpec(memory_space=pl.ANY)
    o = pl.pallas_call(
        kernel,
        in_specs=[hbm, hbm, hbm],
        out_specs=hbm,
        out_shape=jax.ShapeDtypeStruct((num_groups, M, R, D), q.dtype),
        scratch_shapes=[
            pltpu.VMEM((nb, n, Sq, D), q.dtype),
            pltpu.VMEM((nb, n, Sk, D), k.dtype),
            pltpu.VMEM((nb, n, Sk, D), v.dtype),
            pltpu.VMEM((num_groups, M, R, D), q.dtype),
            pltpu.SemaphoreType.DMA((nb,)),
            pltpu.SemaphoreType.DMA((1,)),
        ],
        compiler_params=pltpu.CompilerParams(
            vmem_limit_bytes=64 * 1024 * 1024),
    )(q3, k3, v3)
    return o.reshape(B, H, Sq, D)
```

```python
import jax
import jax.numpy as jnp
import jax.experimental.pallas as pl
import jax.experimental.pallas.tpu as pltpu

_LOG2E = 1.4426950408889634

_HEADS_PER_CHUNK = 2
_NUM_SLOTS = 4
_PIECE_ROWS = 32
_NUM_PASSES = 256


def _attention_head(q, k, v, scale):
    s = jax.lax.dot_general(
        q, k, (((1,), (1,)), ((), ())), preferred_element_type=jnp.float32)
    m = jnp.max(s, axis=-1, keepdims=True)
    p = jnp.exp2((s - m) * (scale * _LOG2E))
    l = jnp.sum(p, axis=-1, keepdims=True)
    o = jnp.dot(p.astype(v.dtype), v, preferred_element_type=jnp.float32)
    return (o * pl.reciprocal(l, approx=False)).astype(q.dtype)


@jax.jit
def pallas_standalone__mha_softmax__near_ridge_kernel(
    q: jax.Array,
    k: jax.Array,
    v: jax.Array,
):
    B, H, Sq, D = q.shape
    Sk = k.shape[2]
    scale = D ** -0.5
    num_heads = B * H
    n, nb = _HEADS_PER_CHUNK, _NUM_SLOTS
    R, M = _PIECE_ROWS, _NUM_PASSES

    num_chunks = num_heads // n
    pieces_per_head = Sq // R
    heads_per_group = M // pieces_per_head
    num_groups = num_heads // heads_per_group
    assert num_heads % n == 0 and Sq % R == 0 and M % pieces_per_head == 0
    assert num_heads % heads_per_group == 0 and num_chunks >= nb

    start_step = num_chunks - 2
    heads_done = start_step * n
    early_passes = min(
        M, (heads_done - (num_heads - heads_per_group)) * pieces_per_head)
    assert early_passes >= 1

    q3 = q.reshape(num_heads, Sq, D)
    k3 = k.reshape(num_heads, Sk, D)
    v3 = v.reshape(num_heads, Sk, D)

    def kernel(q_hbm, k_hbm, v_hbm, o_hbm, qb, kb, vb, ob, in_sems, out_sem):
        def reads(step, slot):
            return [
                pltpu.make_async_copy(
                    src.at[pl.ds(step * n, n)], dst.at[slot], in_sems.at[slot])
                for src, dst in ((q_hbm, qb), (k_hbm, kb), (v_hbm, vb))
            ]

        def start_write_passes(lo, hi):
            @pl.loop(lo, hi)
            def _(j):
                pltpu.make_async_copy(
                    ob.at[:, j], o_hbm.at[:, j], out_sem.at[0]).start()

        for i in range(nb - 1):
            for c in reads(i, i):
                c.start()

        @pl.loop(0, num_chunks)
        def _(i):
            @pl.when(i + nb - 1 < num_chunks)
            def _():
                for c in reads(i + nb - 1, (i + nb - 1) % nb):
                    c.start()

            slot = i % nb
            for c in reads(i, slot):
                c.wait()

            @pl.when(i == start_step)
            def _():
                start_write_passes(0, early_passes)

            for h in range(n):
                head = i * n + h
                o = _attention_head(
                    qb[slot, h], kb[slot, h], vb[slot, h], scale)
                ob[head // heads_per_group,
                   pl.ds((head % heads_per_group) * pieces_per_head,
                         pieces_per_head)] = o.reshape(pieces_per_head, R, D)

        if early_passes < M:
            start_write_passes(early_passes, M)
        pltpu.make_async_copy(ob, o_hbm, out_sem.at[0]).wait()

    hbm = pl.BlockSpec(memory_space=pl.ANY)
    o = pl.pallas_call(
        kernel,
        in_specs=[hbm, hbm, hbm],
        out_specs=hbm,
        out_shape=jax.ShapeDtypeStruct((num_groups, M, R, D), q.dtype),
        scratch_shapes=[
            pltpu.VMEM((nb, n, Sq, D), q.dtype),
            pltpu.VMEM((nb, n, Sk, D), k.dtype),
            pltpu.VMEM((nb, n, Sk, D), v.dtype),
            pltpu.VMEM((num_groups, M, R, D), q.dtype),
            pltpu.SemaphoreType.DMA((nb,)),
            pltpu.SemaphoreType.DMA((1,)),
        ],
        compiler_params=pltpu.CompilerParams(
            vmem_limit_bytes=64 * 1024 * 1024),
    )(q3, k3, v3)
    return o.reshape(B, H, Sq, D)
```

```python
import jax
import jax.numpy as jnp
import jax.experimental.pallas as pl
import jax.experimental.pallas.tpu as pltpu

_LOG2E = 1.4426950408889634

_HEADS_PER_CHUNK = 4
_NUM_SLOTS = 3
_PIECE_ROWS = 32
_NUM_PASSES = 256
_WRITE_START_HEAD = 3


def _attention_head(q, k, v, scale):
    s = jax.lax.dot_general(
        q, k, (((1,), (1,)), ((), ())), preferred_element_type=jnp.float32)
    m = jnp.max(s, axis=-1, keepdims=True)
    p = jnp.exp2((s - m) * (scale * _LOG2E))
    l = jnp.sum(p, axis=-1, keepdims=True)
    o = jnp.dot(p.astype(v.dtype), v, preferred_element_type=jnp.float32)
    return (o * pl.reciprocal(l, approx=False)).astype(q.dtype)


@jax.jit
def pallas_standalone__mha_softmax__near_ridge_kernel(
    q: jax.Array,
    k: jax.Array,
    v: jax.Array,
):
    B, H, Sq, D = q.shape
    Sk = k.shape[2]
    scale = D ** -0.5
    num_heads = B * H
    n, nb = _HEADS_PER_CHUNK, _NUM_SLOTS
    R, M = _PIECE_ROWS, _NUM_PASSES

    num_chunks = num_heads // n
    pieces_per_head = Sq // R
    heads_per_group = M // pieces_per_head
    num_groups = num_heads // heads_per_group
    assert num_heads % n == 0 and Sq % R == 0 and M % pieces_per_head == 0
    assert num_heads % heads_per_group == 0 and num_chunks >= nb >= 3

    start_chunk = num_chunks - 2
    heads_done = start_chunk * n + _WRITE_START_HEAD
    early_passes = min(
        M, (heads_done - (num_heads - heads_per_group)) * pieces_per_head)
    assert early_passes >= 1

    q3 = q.reshape(num_heads, Sq, D)
    k3 = k.reshape(num_heads, Sk, D)
    v3 = v.reshape(num_heads, Sk, D)

    def kernel(q_hbm, k_hbm, v_hbm, o_hbm, qb, kb, vb, ob, in_sems, out_sem):
        def reads(chunk, slot):
            return [
                pltpu.make_async_copy(
                    src.at[pl.ds(chunk * n, n)], dst.at[slot], in_sems.at[slot])
                for src, dst in ((q_hbm, qb), (k_hbm, kb), (v_hbm, vb))
            ]

        def start_write_passes(lo, hi):
            @pl.loop(lo, hi)
            def _(j):
                pltpu.make_async_copy(
                    ob.at[:, j], o_hbm.at[:, j], out_sem.at[0]).start()

        def compute(chunk, h):
            slot = chunk % nb
            head = chunk * n + h
            o = _attention_head(qb[slot, h], kb[slot, h], vb[slot, h], scale)
            ob[head // heads_per_group,
               pl.ds((head % heads_per_group) * pieces_per_head,
                     pieces_per_head)] = o.reshape(pieces_per_head, R, D)

        for i in range(nb - 1):
            for c in reads(i, i):
                c.start()

        num_steady = num_chunks - (nb - 1)

        @pl.loop(0, num_steady)
        def _(i):
            for c in reads(i + nb - 1, (i + nb - 1) % nb):
                c.start()
            for c in reads(i, i % nb):
                c.wait()
            for h in range(n):
                compute(i, h)

        for i in range(num_steady, num_chunks):
            for c in reads(i, i % nb):
                c.wait()
            for h in range(n):
                if i == start_chunk and h == _WRITE_START_HEAD:
                    start_write_passes(0, early_passes)
                compute(i, h)

        if early_passes < M:
            start_write_passes(early_passes, M)
        pltpu.make_async_copy(ob, o_hbm, out_sem.at[0]).wait()

    hbm = pl.BlockSpec(memory_space=pl.ANY)
    o = pl.pallas_call(
        kernel,
        in_specs=[hbm, hbm, hbm],
        out_specs=hbm,
        out_shape=jax.ShapeDtypeStruct((num_groups, M, R, D), q.dtype),
        scratch_shapes=[
            pltpu.VMEM((nb, n, Sq, D), q.dtype),
            pltpu.VMEM((nb, n, Sk, D), k.dtype),
            pltpu.VMEM((nb, n, Sk, D), v.dtype),
            pltpu.VMEM((num_groups, M, R, D), q.dtype),
            pltpu.SemaphoreType.DMA((nb,)),
            pltpu.SemaphoreType.DMA((1,)),
        ],
        compiler_params=pltpu.CompilerParams(
            vmem_limit_bytes=64 * 1024 * 1024),
    )(q3, k3, v3)
    return o.reshape(B, H, Sq, D)
```
